```python
import os as _os
_os.environ.setdefault('JAX_PLATFORMS', 'cpu')
import jax
import jax.numpy as jnp

def _softmax(x, axis=-1):
    return jax.nn.softmax(x, axis=axis)

def _gelu(x):
    return jax.nn.gelu(x, approximate=True)

def _silu(x):
    return jax.nn.silu(x)

def _sigmoid(x):
    return jax.nn.sigmoid(x)

def _layernorm(x, axis=-1, eps=1e-05):
    m = jnp.mean(x, axis=axis, keepdims=True)
    v = jnp.var(x, axis=axis, keepdims=True)
    return (x - m) / jnp.sqrt(v + eps)

def _scatter_add(tgt, idx, src, axis=0):
    return tgt.at[idx].add(src)

def _segment_sum(src, seg, n):
    return jax.ops.segment_sum(src, seg, n)

class _Rng:

    def __init__(self, key):
        self._k = key

    def _next(self):
        self._k, sub = jax.random.split(self._k)
        return sub

    def normal(self, shape):
        return jax.random.normal(self._next(), shape, dtype=jnp.bfloat16)

    def randint(self, lo, hi, shape):
        return jax.random.randint(self._next(), shape, lo, hi, dtype=jnp.int32)

    def uniform(self, shape, lo=0.0, hi=1.0):
        return jax.random.uniform(self._next(), shape, jnp.bfloat16, lo, hi)

    def permutation(self, n):
        return jax.random.permutation(self._next(), n)
kernel_name = 'adaLN_cond__mha_block__dense_activation_squared_relu__prompt'

def setup_inputs():
    _rng = _Rng(jax.random.key(int.from_bytes(__import__("os").urandom(4), "little")))
    _w = lambda a: (lambda t: t.astype(jnp.bfloat16) if jnp.issubdtype(t.dtype, jnp.floating) else t)(jnp.asarray(a))

    def _A_setup():
        B, S, D, H = (1, 2048, 512, 32)
        return {'x': _w((lambda *s: _rng.normal(s) * 0.05)(B, S, D)), 'wqkv': _w((lambda *s: _rng.normal(s) * 0.1)(D, 3 * D)), 'wo': _w((lambda *s: _rng.normal(s) * 0.05)(D, D))}
    _A_in = _A_setup()

    def _B_setup():
        B, S, D, F = (1, 2048, 512, 1792)
        return {'x': _w((lambda *s: _rng.normal(s) * 0.05)(B, S, D)), 'w1': _w((lambda *s: _rng.normal(s) * 0.05)(D, F)), 'b1': _w((lambda *s: _rng.normal(s) * 0.05)(F)), 'w2': _w((lambda *s: _rng.normal(s) * 0.05)(F, D)), 'b2': _w((lambda *s: _rng.normal(s) * 0.05)(D))}
    _B_in = _B_setup()
    return {'A_x': _A_in['x'], 'A_wqkv': _A_in['wqkv'], 'A_wo': _A_in['wo'], 'B_x': _B_in['x'], 'B_w1': _B_in['w1'], 'B_b1': _B_in['b1'], 'B_w2': _B_in['w2'], 'B_b2': _B_in['b2'], 'c': _w((lambda *s: _rng.normal(s) * 0.05)(1, 512) * 8.0), 'w_mod': _w((lambda *s: _rng.normal(s) * 0.05)(512, 6 * 512) * 512 ** (-0.5) * 8.0)}

def reference(A_x, A_wqkv, A_wo, B_x, B_w1, B_b1, B_w2, B_b2, c, w_mod):

    def _A_ref(x, wqkv, wo):
        B, S, D = x.shape
        H = 32
        Dh = D // H
        qkv = (lambda x, *d: x.transpose(*d))((x @ wqkv).reshape(B, S, 3, H, Dh), 2, 0, 3, 1, 4)
        q, k, v = (qkv[0], qkv[1], qkv[2])
        scores = jnp.einsum('bhqd,bhkd->bhqk', q, k) * Dh ** (-0.5)
        p = _softmax(scores, axis=-1)
        o = jnp.einsum('bhqk,bhkd->bhqd', p, v)
        return (lambda x, *d: x.transpose(*d))(o, 0, 2, 1, 3).reshape(B, S, D) @ wo

    def _B_ref(x, w1, b1, w2, b2):
        h = jnp.einsum('bsd,df->bsf', x, w1) + b1
        zero = jnp.zeros_like(h)
        r = jnp.where(h > zero, h, zero)
        h = r * r
        out = jnp.einsum('bsf,fd->bsd', h, w2) + b2
        return out
    x = A_x
    mod = (_silu(c) @ w_mod).reshape(c.shape[0], 6, 1, -1)
    sa, ca, ga, sb, cb, gb = (mod[:, 0].copy(), mod[:, 1].copy(), mod[:, 2].copy(), mod[:, 3].copy(), mod[:, 4].copy(), mod[:, 5].copy())
    h = _layernorm(x, axis=-1) * (1 + ca) + sa
    x = x + ga * _A_ref(h, A_wqkv, A_wo)
    h = _layernorm(x, axis=-1) * (1 + cb) + sb
    x = x + gb * _B_ref(h, B_w1, B_b1, B_w2, B_b2)
    return x
```

```python
import numpy as np
import jax
import jax.numpy as jnp
from jax import lax
import jax.experimental.pallas as pl
import jax.experimental.pallas.tpu as pltpu

S, D, H, DH, F = 2048, 512, 32, 16, 1792
LOG2E = 1.4426950408889634
BF, F32 = jnp.bfloat16, jnp.float32

BQ, BK, UNR = 1024, 128, 2
TC1, TC3 = 512, 512
STAGE = 0
SCOPES = 0
L_LO, L_HI, A_HI = 2.0 ** -40, 2.0 ** 100, 2.0 ** 120
N1, N3 = S // TC1, S // TC3


class _nul:
    def __enter__(s): pass
    def __exit__(s, *a): pass


def scope(n):
    return jax.named_scope(n) if SCOPES else _nul()


def _ln(x):
    m = jnp.mean(x, axis=-1, keepdims=True)
    xc = x - m
    v = jnp.mean(xc * xc, axis=-1, keepdims=True)
    return xc * lax.rsqrt(v + 1e-5)


def _nt(a, b):
    return lax.dot_general(a, b, (((1,), (1,)), ((), ())), preferred_element_type=F32)


def _silu_rows(c_ref):
    cc = jnp.broadcast_to(c_ref[...].astype(F32), (8, D))
    return (cc * jax.nn.sigmoid(cc)).astype(BF)


def _kernel(x_hbm, wqkv_hbm, wo_hbm, w1_hbm, b1_hbm, w2_hbm, b2_hbm, c_hbm, wmod_hbm,
            out_hbm,
            xb, wq, wk, wv, wo, w1, b1b, w2, b2b, cb, wma, wmb, ob,
            hbuf, kbuf, qT, vT, oT, modb, pcar, lcar, sems, osems):
    def cp(i, src, dst):
        return pltpu.make_async_copy(src, dst, sems.at[i])

    c_cp = cp(0, c_hbm, cb)
    wma_cp = cp(1, wmod_hbm.at[:, pl.ds(0, 2 * D)], wma)
    wk_cp = cp(2, wqkv_hbm.at[:, pl.ds(D, D)], wk)
    wq_cp = cp(3, wqkv_hbm.at[:, pl.ds(0, D)], wq)
    wv_cp = cp(4, wqkv_hbm.at[:, pl.ds(2 * D, D)], wv)
    rest = [cp(5, wmod_hbm.at[:, pl.ds(2 * D, 4 * D)], wmb), cp(6, wo_hbm, wo), cp(7, w1_hbm, w1),
            cp(8, w2_hbm, w2), cp(9, b1_hbm, b1b), cp(10, b2_hbm, b2b)]
    x_cp = [cp(11 + t, x_hbm.at[pl.ds(t * TC1, TC1)], xb.at[pl.ds(t * TC1, TC1)]) for t in range(N1)]

    c_cp.start()
    x_cp[0].start()
    wma_cp.start()
    wk_cp.start()
    if STAGE == 0:
        for t in range(1, N1):
            x_cp[t].start()
        wq_cp.start()
        wv_cp.start()
        for r in rest:
            r.start()

    with scope("p1"):
        c_cp.wait()
        x_cp[0].wait()
        if STAGE == 1:
            for t in range(1, N1):
                x_cp[t].start()
            wq_cp.start()
            wv_cp.start()
        elif STAGE == 2:
            for t in range(1, N1):
                x_cp[t].start()
        xn = _ln(xb[0:TC1, :].astype(F32))
        wma_cp.wait()
        mod = jnp.dot(_silu_rows(cb), wma[...], preferred_element_type=F32)
        sa = mod[0:1, 0:D]
        ca1 = mod[0:1, D:2 * D] + 1.0
        wk_cp.wait()
        if STAGE == 1:
            for r in rest:
                r.start()
        elif STAGE == 2:
            wq_cp.start()
            wv_cp.start()
        for t in range(N1):
            rows = slice(t * TC1, (t + 1) * TC1)
            h = (xn * ca1 + sa).astype(BF)
            hbuf[rows, :] = h
            if t + 1 < N1:
                x_cp[t + 1].wait()
                xn = _ln(xb[(t + 1) * TC1:(t + 2) * TC1, :].astype(F32))
            k = jnp.dot(h, wk[...], preferred_element_type=F32).astype(BF)
            for g in range(4):
                kbuf[g, rows, :] = k[:, g * 128:(g + 1) * 128]
        wq_cp.wait()
        wv_cp.wait()
        if STAGE == 2:
            for r in rest:
                r.start()
        wqT = wq[...].astype(F32).T.astype(BF)
        wvT = wv[...].astype(F32).T.astype(BF)
        for t in range(N1):
            rows = slice(t * TC1, (t + 1) * TC1)
            h = hbuf[rows, :]
            qT[:, rows] = (_nt(wqT, h) * (LOG2E * DH ** -0.5)).astype(BF)
            vT[:, rows] = _nt(wvT, h).astype(BF)

    rowgrp = lax.broadcasted_iota(jnp.int32, (128, BQ), 0) // DH
    NK = S // BK
    NB = S // BQ
    steps = [(b, kk) for b in range(NB) for kk in range(NK)]

    def qsel(h, b):
        g0 = pl.multiple_of((h // 8) * 128, 128)
        blk = qT[pl.ds(g0, 128), b * BQ:(b + 1) * BQ]
        return jnp.where(rowgrp == h % 8, blk.astype(F32), 0.0).astype(BF)

    def qk(h, kk, q):
        return jnp.dot(kbuf[h // 8, kk * BK:(kk + 1) * BK, :], q, preferred_element_type=F32)

    def lsum(p):
        return jnp.sum(p.reshape(BK // 8, 8, BQ), axis=0)

    def heads(it, bad):
        pb = pcar[...]
        l = lcar[...]
        for u in range(UNR):
            h = it * UNR + u
            hn = jnp.minimum(h + 1, H - 1)
            r0 = pl.multiple_of(h * DH, DH)
            q = qsel(h, 0)
            acc = None
            for t, (b, kk) in enumerate(steps):
                nh, (nb, nk) = (h, steps[t + 1]) if t + 1 < len(steps) else (hn, (0, 0))
                if nk == 0:
                    q = qsel(nh, nb)
                s = qk(nh, nk, q)
                d = jnp.dot(vT[pl.ds(r0, DH), kk * BK:(kk + 1) * BK], pb, preferred_element_type=F32)
                acc = d if kk == 0 else acc + d
                if kk == NK - 1:
                    lt = jnp.sum(l, axis=0, keepdims=True)
                    am = jnp.max(jnp.abs(acc), axis=0, keepdims=True)
                    ok = (lt >= L_LO) & (lt <= L_HI) & (am <= A_HI)
                    bad = jnp.maximum(bad, jnp.where(ok, 0.0, 1.0))
                    oT[pl.ds(r0, DH), b * BQ:(b + 1) * BQ] = (acc * (1.0 / lt)).astype(BF)
                p = jnp.exp2(s)
                l = lsum(p) if nk == 0 else l + lsum(p)
                pb = p.astype(BF)
        pcar[...] = pb
        lcar[...] = l
        return bad

    with scope("p2"):
        p0 = jnp.exp2(qk(0, 0, qsel(0, 0)))
        pcar[...] = p0.astype(BF)
        lcar[...] = lsum(p0)
        bad = lax.fori_loop(0, H // UNR, heads, jnp.zeros((1, BQ), F32))

    @pl.when(jnp.max(bad) > 0.0)
    def _slow():
        SB = 256
        rg = lax.broadcasted_iota(jnp.int32, (128, SB), 0) // DH

        def blk(i, carry):
            h = i // (S // SB)
            c0 = pl.multiple_of((i % (S // SB)) * SB, SB)
            g = h // 8
            r0 = pl.multiple_of(h * DH, DH)
            g0 = pl.multiple_of(g * 128, 128)
            q = jnp.where(rg == h % 8, qT[pl.ds(g0, 128), pl.ds(c0, SB)].astype(F32), 0.0).astype(BF)
            s = jnp.dot(kbuf[g], q, preferred_element_type=F32)
            m = jnp.max(s, axis=0, keepdims=True)
            p = jnp.exp2(s - m)
            l = jnp.sum(p, axis=0, keepdims=True)
            acc = jnp.dot(vT[pl.ds(r0, DH), :], p.astype(BF), preferred_element_type=F32)
            oT[pl.ds(r0, DH), pl.ds(c0, SB)] = (acc / l).astype(BF)
            return carry

        lax.fori_loop(0, H * (S // SB), blk, 0)

    with scope("p3"):
        for r in rest:
            r.wait()
        mod2 = jnp.dot(_silu_rows(cb), wmb[...], preferred_element_type=F32)
        ga = mod2[0:1, 0:D]
        sb = mod2[0:1, D:2 * D]
        cb1 = mod2[0:1, 2 * D:3 * D] + 1.0
        gb = mod2[0:1, 3 * D:4 * D]
        b1 = b1b[...].astype(F32).reshape(1, F)
        b2 = b2b[...].astype(F32).reshape(1, D)
        ocp = []
        for t in range(N3):
            rows = slice(t * TC3, (t + 1) * TC3)
            a = lax.dot_general(oT[:, rows], wo[...], (((0,), (0,)), ((), ())),
                                preferred_element_type=F32)
            x1 = xb[rows, :].astype(F32) + ga * a
            h2 = (_ln(x1) * cb1 + sb).astype(BF)
            u = jnp.dot(h2, w1[...], preferred_element_type=F32) + b1
            r = jnp.maximum(u, 0.0)
            f = jnp.dot((r * r).astype(BF), w2[...], preferred_element_type=F32) + b2
            ob[rows, :] = (x1 + gb * f).astype(BF)
            o = pltpu.make_async_copy(ob.at[pl.ds(t * TC3, TC3)], out_hbm.at[pl.ds(t * TC3, TC3)], osems.at[t])
            o.start()
            ocp.append(o)
        for o in ocp:
            o.wait()


@jax.jit
def pallas_adaLN_cond__mha_block__dense_activation_squared_relu__prompt_kernel(A_x, A_wqkv, A_wo, B_x, B_w1, B_b1, B_w2, B_b2, c, w_mod):
    del B_x
    anyspec = pl.BlockSpec(memory_space=pl.ANY)
    V = pltpu.VMEM
    out = pl.pallas_call(
        _kernel,
        out_shape=jax.ShapeDtypeStruct((S, D), A_x.dtype),
        in_specs=[anyspec] * 9,
        out_specs=anyspec,
        scratch_shapes=[
            V((S, D), BF), V((D, D), BF), V((D, D), BF), V((D, D), BF), V((D, D), BF),
            V((D, F), BF), V((F,), BF), V((F, D), BF), V((D,), BF), V((1, D), BF),
            V((D, 2 * D), BF), V((D, 4 * D), BF), V((S, D), BF),
            V((S, D), BF), V((4, S, 128), BF), V((D, S), BF), V((D, S), BF), V((D, S), BF),
            V((8, 6 * D), F32), V((BK, BQ), BF), V((8, BQ), F32),
            pltpu.SemaphoreType.DMA((11 + N1,)), pltpu.SemaphoreType.DMA((N3,)),
        ],
        compiler_params=pltpu.CompilerParams(vmem_limit_bytes=100 * 2 ** 20),
    )(A_x.reshape(S, D), A_wqkv, A_wo, B_w1, B_b1, B_w2, B_b2, c, w_mod)
    return out.reshape(1, S, D)
```

```python
import jax
import jax.numpy as jnp
from jax import lax
import jax.experimental.pallas as pl
import jax.experimental.pallas.tpu as pltpu

S, D, H, DH, F = 2048, 512, 32, 16, 1792
LOG2E = 1.4426950408889634
BF, F32 = jnp.bfloat16, jnp.float32

BQ, BK, UNR = 1024, 128, 2
KD = 32
KPAD = 32
L_LO, L_HI, A_HI = 2.0 ** -20, 2.0 ** 100, 2.0 ** 120


def _ranges(sizes):
    return [(sum(sizes[:i]), sum(sizes[:i + 1])) for i in range(len(sizes))]


C1 = _ranges([256, 256, 768, 768])
C3 = _ranges([128, 640, 640, 512, 128])
SCHED1 = "h0 k0 h1 k1 tq q0 tv q1 v0 h2 v1 k2 q2 h3 v2 k3 q3 v3".split()


def _ln(x):
    m = jnp.mean(x, axis=-1, keepdims=True)
    xc = x - m
    v = jnp.mean(xc * xc, axis=-1, keepdims=True)
    return xc * lax.rsqrt(v + 1e-5)


def _nt(a, b):
    return lax.dot_general(a, b, (((1,), (1,)), ((), ())), preferred_element_type=F32)


def _silu_rows(c_ref):
    cc = jnp.broadcast_to(c_ref[...].astype(F32), (8, D))
    return (cc * jax.nn.sigmoid(cc)).astype(BF)


def _kernel(x_hbm, wqkv_hbm, wo_hbm, w1_hbm, b1_hbm, w2_hbm, b2_hbm, c_hbm, wmod_hbm,
            out_hbm,
            xb, wq, wk, wv, wo, w1, b1b, w2, b2b, cb, wma, wmb, ob,
            x1b, hbuf, kbuf, qT, vT, oT, pcar, lcar, sems, osems):
    def cp(i, src, dst):
        return pltpu.make_async_copy(src, dst, sems.at[i])

    c_cp = cp(0, c_hbm, cb)
    wma_cp = cp(1, wmod_hbm.at[:, pl.ds(0, 2 * D)], wma)
    wk_cp = cp(2, wqkv_hbm.at[:, pl.ds(D, D)], wk)
    wq_cp = cp(3, wqkv_hbm.at[:, pl.ds(0, D)], wq)
    wv_cp = cp(4, wqkv_hbm.at[:, pl.ds(2 * D, D)], wv)
    rest = [cp(5, wmod_hbm.at[:, pl.ds(2 * D, 4 * D)], wmb), cp(6, wo_hbm, wo), cp(7, w1_hbm, w1),
            cp(8, w2_hbm, w2), cp(9, b1_hbm, b1b), cp(10, b2_hbm, b2b)]
    x_cp = [cp(11 + t, x_hbm.at[pl.ds(a, b - a)], xb.at[pl.ds(a, b - a)])
            for t, (a, b) in enumerate(C1)]

    for d in (c_cp, x_cp[0], wma_cp, wk_cp, x_cp[1], wq_cp, wv_cp):
        d.start()

    c_cp.wait()
    x_cp[0].wait()
    xn0 = _ln(xb[slice(*C1[0]), :].astype(F32))
    wma_cp.wait()
    for d in x_cp[2:]:
        d.start()
    mod = jnp.dot(_silu_rows(cb), wma[...], preferred_element_type=F32)
    sa = mod[0:1, 0:D]
    ca1 = mod[0:1, D:2 * D] + 1.0
    wk_cp.wait()
    wT = {}

    def mk_h(t):
        r = slice(*C1[t])
        if t > 0:
            x_cp[t].wait()
        xn = _ln(xb[r, :].astype(F32)) if t > 0 else xn0
        hbuf[r, :] = (xn * ca1 + sa).astype(BF)

    def mk_k(t):
        r = slice(*C1[t])
        k = jnp.dot(hbuf[r, :], wk[...], preferred_element_type=F32).astype(BF)
        for g in range(4):
            kg = k[:, g * 128:(g + 1) * 128]
            kbuf[g * (128 // KD), r, :] = kg
            for j in range(1, 128 // KD):
                u = pltpu.roll(pltpu.bitcast(kg, jnp.uint32), 128 - KD * j, 1)
                kbuf[g * (128 // KD) + j, r, :] = pltpu.bitcast(u, BF)

    def mk_q(t):
        r = slice(*C1[t])
        qT[:, r] = (_nt(wT["q"], hbuf[r, :]) * (LOG2E * DH ** -0.5)).astype(BF)

    def mk_v(t):
        r = slice(*C1[t])
        vT[:, r] = _nt(wT["v"], hbuf[r, :]).astype(BF)

    for tok in SCHED1:
        if tok == "tq":
            wq_cp.wait()
            wT["q"] = wq[...].astype(F32).T.astype(BF)
        elif tok == "tv":
            wv_cp.wait()
            for d in rest:
                d.start()
            wT["v"] = wv[...].astype(F32).T.astype(BF)
        else:
            {"h": mk_h, "k": mk_k, "q": mk_q, "v": mk_v}[tok[0]](int(tok[1:]))

    HG = KD // DH
    NK, NB = S // BK, S // BQ
    steps = [(b, kk) for b in range(NB) for kk in range(NK)]
    rowgrp = lax.broadcasted_iota(jnp.int32, (KD, BQ), 0) // DH

    def qsel(h, b):
        g0 = pl.multiple_of((h // HG) * KD, KD)
        blk = qT[pl.ds(g0, KD), b * BQ:(b + 1) * BQ]
        return jnp.where(rowgrp == h % HG, blk.astype(F32), 0.0).astype(BF)

    def qk(h, kk, q):
        return jnp.dot(kbuf[h // HG, kk * BK:(kk + 1) * BK, 0:KD], q, preferred_element_type=F32)

    def lsum(p):
        return jnp.sum(p.reshape(BK // 8, 8, BQ), axis=0)

    def heads(it, bad):
        pb = pcar[...]
        l = lcar[...]
        for u in range(UNR):
            h = it * UNR + u
            hn = jnp.minimum(h + 1, H - 1)
            r0 = pl.multiple_of(h * DH, DH)
            q = qsel(h, 0)
            acc = None
            for t, (b, kk) in enumerate(steps):
                nh, (nb, nk) = (h, steps[t + 1]) if t + 1 < len(steps) else (hn, (0, 0))
                if nk == 0:
                    q = qsel(nh, nb)
                s = qk(nh, nk, q)
                d = jnp.dot(vT[pl.ds(r0, DH), kk * BK:(kk + 1) * BK], pb,
                            preferred_element_type=F32)
                acc = d if kk == 0 else acc + d
                if kk == NK - 1:
                    lt = jnp.sum(l, axis=0, keepdims=True)
                    oT[pl.ds(r0, DH), b * BQ:(b + 1) * BQ] = (acc * (1.0 / lt)).astype(BF)
                    am = jnp.max(jnp.abs(acc), axis=0, keepdims=True)
                    ok = (lt >= L_LO) & (lt <= L_HI) & (am <= A_HI)
                    bad = jnp.maximum(bad, jnp.where(ok, 0.0, 1.0))
                p = jnp.exp2(s)
                l = lsum(p) if nk == 0 else l + lsum(p)
                pb = p.astype(BF)
        pcar[...] = pb
        lcar[...] = l
        return bad

    p0 = jnp.exp2(qk(0, 0, qsel(0, 0)))
    pcar[...] = p0.astype(BF)
    lcar[...] = lsum(p0)
    bad = lax.fori_loop(0, H // UNR, heads, jnp.zeros((1, BQ), F32))

    @pl.when(jnp.max(bad) > 0.0)
    def _shifted_softmax():
        SB = 256
        rg = lax.broadcasted_iota(jnp.int32, (128, SB), 0) // DH

        def blk(i, carry):
            h = i // (S // SB)
            c0 = pl.multiple_of((i % (S // SB)) * SB, SB)
            g = h // 8
            r0 = pl.multiple_of(h * DH, DH)
            g0 = pl.multiple_of(g * 128, 128)
            q = jnp.where(rg == h % 8, qT[pl.ds(g0, 128), pl.ds(c0, SB)].astype(F32), 0.0).astype(BF)
            s = jnp.dot(kbuf[g * (128 // KD), 0:S, :], q, preferred_element_type=F32)
            m = jnp.max(s, axis=0, keepdims=True)
            p = jnp.exp2(s - m)
            l = jnp.sum(p, axis=0, keepdims=True)
            acc = jnp.dot(vT[pl.ds(r0, DH), :], p.astype(BF), preferred_element_type=F32)
            oT[pl.ds(r0, DH), pl.ds(c0, SB)] = (acc / l).astype(BF)
            return carry

        lax.fori_loop(0, H * (S // SB), blk, 0)

    for d in rest:
        d.wait()
    mod2 = jnp.dot(_silu_rows(cb), wmb[...], preferred_element_type=F32)
    ga = mod2[0:1, 0:D]
    sb = mod2[0:1, D:2 * D]
    cb1 = mod2[0:1, 2 * D:3 * D] + 1.0
    gb = mod2[0:1, 3 * D:4 * D]
    b1 = b1b[...].astype(F32).reshape(1, F)
    b2 = b2b[...].astype(F32).reshape(1, D)
    out_cp = []

    def pre(t):
        r = slice(*C3[t])
        a = lax.dot_general(oT[:, r], wo[...], (((0,), (0,)), ((), ())),
                            preferred_element_type=F32)
        x1 = xb[r, :].astype(F32) + ga * a
        x1b[r, :] = x1
        hbuf[r, :] = (_ln(x1) * cb1 + sb).astype(BF)

    def ffn(t):
        r = slice(*C3[t])
        u = jnp.dot(hbuf[r, :], w1[...], preferred_element_type=F32) + b1
        rl = jnp.maximum(u, 0.0)
        f = jnp.dot((rl * rl).astype(BF), w2[...], preferred_element_type=F32) + b2
        ob[r, :] = (x1b[r, :] + gb * f).astype(BF)
        a, b = C3[t]
        o = pltpu.make_async_copy(ob.at[pl.ds(a, b - a)], out_hbm.at[pl.ds(a, b - a)], osems.at[t])
        o.start()
        out_cp.append(o)

    pre(0)
    for t in range(len(C3)):
        if t + 1 < len(C3):
            pre(t + 1)
        ffn(t)
    for o in out_cp:
        o.wait()


@jax.jit
def pallas_adaLN_cond__mha_block__dense_activation_squared_relu__prompt_kernel(
    A_x: jax.Array,
    A_wqkv: jax.Array,
    A_wo: jax.Array,
    B_x: jax.Array,
    B_w1: jax.Array,
    B_b1: jax.Array,
    B_w2: jax.Array,
    B_b2: jax.Array,
    c: jax.Array,
    w_mod: jax.Array,
):
    del B_x
    assert A_x.shape == (1, S, D) and B_w1.shape == (D, F)
    anyspec = pl.BlockSpec(memory_space=pl.ANY)
    V = pltpu.VMEM
    out = pl.pallas_call(
        _kernel,
        out_shape=jax.ShapeDtypeStruct((S, D), A_x.dtype),
        in_specs=[anyspec] * 9,
        out_specs=anyspec,
        scratch_shapes=[
            V((S, D), BF), V((D, D), BF), V((D, D), BF), V((D, D), BF), V((D, D), BF),
            V((D, F), BF), V((F,), BF), V((F, D), BF), V((D,), BF), V((1, D), BF),
            V((D, 2 * D), BF), V((D, 4 * D), BF), V((S, D), BF),
            V((S, D), F32), V((S, D), BF), V((D // KD, S + KPAD, 128), BF),
            V((D, S), BF), V((D, S), BF), V((D, S), BF),
            V((BK, BQ), BF), V((8, BQ), F32),
            pltpu.SemaphoreType.DMA((11 + len(C1),)), pltpu.SemaphoreType.DMA((len(C3),)),
        ],
        compiler_params=pltpu.CompilerParams(vmem_limit_bytes=100 * 2 ** 20),
    )(A_x.reshape(S, D), A_wqkv, A_wo, B_w1, B_b1, B_w2, B_b2, c, w_mod)
    return out.reshape(1, S, D)
```

```python
import jax
import jax.numpy as jnp
from jax import lax
import jax.experimental.pallas as pl
import jax.experimental.pallas.tpu as pltpu

S, D, H, DH, F = 2048, 512, 32, 16, 1792
LOG2E = 1.4426950408889634
BF, F32 = jnp.bfloat16, jnp.float32

BQ, BK, UNR = 1024, 128, 2
KD = 32
KPAD = 32
L_LO, L_HI, A_HI = 2.0 ** -20, 2.0 ** 100, 2.0 ** 120


def _ranges(sizes):
    return [(sum(sizes[:i]), sum(sizes[:i + 1])) for i in range(len(sizes))]


C1 = _ranges([256, 256, 768, 768])
C3 = _ranges([128, 896, 896, 128])
SCHED1 = "h0 k0 h1 k1 tq q0 tv q1 v0 h2 v1 k2 q2 h3 v2 k3 q3 v3".split()


def _ln(x):
    m = jnp.mean(x, axis=-1, keepdims=True)
    xc = x - m
    v = jnp.mean(xc * xc, axis=-1, keepdims=True)
    return xc * lax.rsqrt(v + 1e-5)


def _nt(a, b):
    return lax.dot_general(a, b, (((1,), (1,)), ((), ())), preferred_element_type=F32)


def _silu_rows(c_ref):
    cc = jnp.broadcast_to(c_ref[...].astype(F32), (8, D))
    return (cc * jax.nn.sigmoid(cc)).astype(BF)


def _kernel(x_hbm, wqkv_hbm, wo_hbm, w1_hbm, b1_hbm, w2_hbm, b2_hbm, c_hbm, wmod_hbm,
            out_hbm,
            xb, wq, wk, wv, wo, w1, b1b, w2, b2b, cb, wma, wmb, ob,
            x1b, hbuf, kbuf, qT, vT, oT, pcar, lcar, sems, osems):
    def cp(i, src, dst):
        return pltpu.make_async_copy(src, dst, sems.at[i])

    c_cp = cp(0, c_hbm, cb)
    wma_cp = cp(1, wmod_hbm.at[:, pl.ds(0, 2 * D)], wma)
    wk_cp = cp(2, wqkv_hbm.at[:, pl.ds(D, D)], wk)
    wq_cp = cp(3, wqkv_hbm.at[:, pl.ds(0, D)], wq)
    wv_cp = cp(4, wqkv_hbm.at[:, pl.ds(2 * D, D)], wv)
    rest = [cp(5, wmod_hbm.at[:, pl.ds(2 * D, 4 * D)], wmb), cp(6, wo_hbm, wo), cp(7, w1_hbm, w1),
            cp(8, w2_hbm, w2), cp(9, b1_hbm, b1b), cp(10, b2_hbm, b2b)]
    x_cp = [cp(11 + t, x_hbm.at[pl.ds(a, b - a)], xb.at[pl.ds(a, b - a)])
            for t, (a, b) in enumerate(C1)]

    for d in (c_cp, x_cp[0], wma_cp, wk_cp, x_cp[1], wq_cp, wv_cp):
        d.start()

    c_cp.wait()
    x_cp[0].wait()
    xn0 = _ln(xb[slice(*C1[0]), :].astype(F32))
    wma_cp.wait()
    for d in x_cp[2:]:
        d.start()
    mod = jnp.dot(_silu_rows(cb), wma[...], preferred_element_type=F32)
    sa = mod[0:1, 0:D]
    ca1 = mod[0:1, D:2 * D] + 1.0
    wk_cp.wait()
    wT = {}

    def mk_h(t):
        r = slice(*C1[t])
        if t > 0:
            x_cp[t].wait()
        xn = _ln(xb[r, :].astype(F32)) if t > 0 else xn0
        hbuf[r, :] = (xn * ca1 + sa).astype(BF)

    def mk_k(t):
        r = slice(*C1[t])
        k = jnp.dot(hbuf[r, :], wk[...], preferred_element_type=F32).astype(BF)
        for g in range(4):
            kg = k[:, g * 128:(g + 1) * 128]
            kbuf[g * (128 // KD), r, :] = kg
            for j in range(1, 128 // KD):
                u = pltpu.roll(pltpu.bitcast(kg, jnp.uint32), 128 - KD * j, 1)
                kbuf[g * (128 // KD) + j, r, :] = pltpu.bitcast(u, BF)

    def mk_q(t):
        r = slice(*C1[t])
        qT[:, r] = (_nt(wT["q"], hbuf[r, :]) * (LOG2E * DH ** -0.5)).astype(BF)

    def mk_v(t):
        r = slice(*C1[t])
        vT[:, r] = _nt(wT["v"], hbuf[r, :]).astype(BF)

    for tok in SCHED1:
        if tok == "tq":
            wq_cp.wait()
            wT["q"] = wq[...].astype(F32).T.astype(BF)
        elif tok == "tv":
            wv_cp.wait()
            for d in rest:
                d.start()
            wT["v"] = wv[...].astype(F32).T.astype(BF)
        else:
            {"h": mk_h, "k": mk_k, "q": mk_q, "v": mk_v}[tok[0]](int(tok[1:]))

    HG = KD // DH
    NK, NB = S // BK, S // BQ
    steps = [(b, kk) for b in range(NB) for kk in range(NK)]
    rowgrp = lax.broadcasted_iota(jnp.int32, (KD, BQ), 0) // DH

    assert UNR == HG

    def qsel(h, b):
        g0 = pl.multiple_of(h[0] * KD, KD)
        blk = qT[pl.ds(g0, KD), b * BQ:(b + 1) * BQ]
        return jnp.where(rowgrp == h[1], blk.astype(F32), 0.0).astype(BF)

    def qk(h, kk, q):
        return jnp.dot(kbuf[h[0], kk * BK:(kk + 1) * BK, 0:KD], q, preferred_element_type=F32)

    def lsum(p):
        return jnp.sum(p.reshape(BK // 8, 8, BQ), axis=0)

    def heads(it, bad):
        pb = pcar[...]
        l = lcar[...]
        for u in range(UNR):
            h = (it, u)
            hn = (it, u + 1) if u + 1 < UNR else (jnp.minimum(it + 1, H // UNR - 1), 0)
            r0 = pl.multiple_of((it * UNR + u) * DH, DH)
            q = qsel(h, 0)
            acc = None
            for t, (b, kk) in enumerate(steps):
                nh, (nb, nk) = (h, steps[t + 1]) if t + 1 < len(steps) else (hn, (0, 0))
                if nk == 0:
                    q = qsel(nh, nb)
                s = qk(nh, nk, q)
                d = jnp.dot(vT[pl.ds(r0, DH), kk * BK:(kk + 1) * BK], pb,
                            preferred_element_type=F32)
                acc = d if kk == 0 else acc + d
                if kk == NK - 1:
                    lt = jnp.sum(l, axis=0, keepdims=True)
                    oT[pl.ds(r0, DH), b * BQ:(b + 1) * BQ] = (acc * (1.0 / lt)).astype(BF)
                    am = jnp.max(jnp.abs(acc), axis=0, keepdims=True)
                    ok = (lt >= L_LO) & (lt <= L_HI) & (am <= A_HI)
                    bad = jnp.maximum(bad, jnp.where(ok, 0.0, 1.0))
                p = jnp.exp2(s)
                l = lsum(p) if nk == 0 else l + lsum(p)
                pb = p.astype(BF)
        pcar[...] = pb
        lcar[...] = l
        return bad

    p0 = jnp.exp2(qk((0, 0), 0, qsel((0, 0), 0)))
    pcar[...] = p0.astype(BF)
    lcar[...] = lsum(p0)
    bad = lax.fori_loop(0, H // UNR, heads, jnp.zeros((1, BQ), F32))

    @pl.when(jnp.max(bad) > 0.0)
    def _shifted_softmax():
        SB = 256
        rg = lax.broadcasted_iota(jnp.int32, (128, SB), 0) // DH

        def blk(i, carry):
            h = i // (S // SB)
            c0 = pl.multiple_of((i % (S // SB)) * SB, SB)
            g = h // 8
            r0 = pl.multiple_of(h * DH, DH)
            g0 = pl.multiple_of(g * 128, 128)
            q = jnp.where(rg == h % 8, qT[pl.ds(g0, 128), pl.ds(c0, SB)].astype(F32), 0.0).astype(BF)
            s = jnp.dot(kbuf[g * (128 // KD), 0:S, :], q, preferred_element_type=F32)
            m = jnp.max(s, axis=0, keepdims=True)
            p = jnp.exp2(s - m)
            l = jnp.sum(p, axis=0, keepdims=True)
            acc = jnp.dot(vT[pl.ds(r0, DH), :], p.astype(BF), preferred_element_type=F32)
            oT[pl.ds(r0, DH), pl.ds(c0, SB)] = (acc / l).astype(BF)
            return carry

        lax.fori_loop(0, H * (S // SB), blk, 0)

    for d in rest:
        d.wait()
    mod2 = jnp.dot(_silu_rows(cb), wmb[...], preferred_element_type=F32)
    ga = mod2[0:1, 0:D]
    sb = mod2[0:1, D:2 * D]
    cb1 = mod2[0:1, 2 * D:3 * D] + 1.0
    gb = mod2[0:1, 3 * D:4 * D]
    b1 = b1b[...].astype(F32).reshape(1, F)
    b2 = b2b[...].astype(F32).reshape(1, D)
    out_cp = []

    def pre(t):
        r = slice(*C3[t])
        a = lax.dot_general(oT[:, r], wo[...], (((0,), (0,)), ((), ())),
                            preferred_element_type=F32)
        x1 = xb[r, :].astype(F32) + ga * a
        x1b[r, :] = x1
        hbuf[r, :] = (_ln(x1) * cb1 + sb).astype(BF)

    def ffn(t):
        r = slice(*C3[t])
        u = jnp.dot(hbuf[r, :], w1[...], preferred_element_type=F32) + b1
        rl = jnp.maximum(u, 0.0)
        f = jnp.dot((rl * rl).astype(BF), w2[...], preferred_element_type=F32) + b2
        ob[r, :] = (x1b[r, :] + gb * f).astype(BF)
        a, b = C3[t]
        o = pltpu.make_async_copy(ob.at[pl.ds(a, b - a)], out_hbm.at[pl.ds(a, b - a)], osems.at[t])
        o.start()
        out_cp.append(o)

    pre(0)
    for t in range(len(C3)):
        if t + 1 < len(C3):
            pre(t + 1)
        ffn(t)
    for o in out_cp:
        o.wait()


@jax.jit
def pallas_adaLN_cond__mha_block__dense_activation_squared_relu__prompt_kernel(
    A_x: jax.Array,
    A_wqkv: jax.Array,
    A_wo: jax.Array,
    B_x: jax.Array,
    B_w1: jax.Array,
    B_b1: jax.Array,
    B_w2: jax.Array,
    B_b2: jax.Array,
    c: jax.Array,
    w_mod: jax.Array,
):
    del B_x
    assert A_x.shape == (1, S, D) and B_w1.shape == (D, F)
    anyspec = pl.BlockSpec(memory_space=pl.ANY)
    V = pltpu.VMEM
    out = pl.pallas_call(
        _kernel,
        out_shape=jax.ShapeDtypeStruct((S, D), A_x.dtype),
        in_specs=[anyspec] * 9,
        out_specs=anyspec,
        scratch_shapes=[
            V((S, D), BF), V((D, D), BF), V((D, D), BF), V((D, D), BF), V((D, D), BF),
            V((D, F), BF), V((F,), BF), V((F, D), BF), V((D,), BF), V((1, D), BF),
            V((D, 2 * D), BF), V((D, 4 * D), BF), V((S, D), BF),
            V((S, D), F32), V((S, D), BF), V((D // KD, S + KPAD, 128), BF),
            V((D, S), BF), V((D, S), BF), V((D, S), BF),
            V((BK, BQ), BF), V((8, BQ), F32),
            pltpu.SemaphoreType.DMA((11 + len(C1),)), pltpu.SemaphoreType.DMA((len(C3),)),
        ],
        compiler_params=pltpu.CompilerParams(vmem_limit_bytes=100 * 2 ** 20),
    )(A_x.reshape(S, D), A_wqkv, A_wo, B_w1, B_b1, B_w2, B_b2, c, w_mod)
    return out.reshape(1, S, D)
```
